```python
import jax
import jax.numpy as jnp

def _softmax(x, axis=-1):
    return jax.nn.softmax(x, axis=axis)

def _gelu(x):
    return jax.nn.gelu(x, approximate=True)

def _silu(x):
    return jax.nn.silu(x)

def _sigmoid(x):
    return jax.nn.sigmoid(x)

def _layernorm(x, axis=-1, eps=1e-05):
    m = jnp.mean(x, axis=axis, keepdims=True)
    v = jnp.var(x, axis=axis, keepdims=True)
    return (x - m) / jnp.sqrt(v + eps)

def _scatter_add(tgt, idx, src, axis=0):
    return tgt.at[idx].add(src)

def _segment_sum(src, seg, n):
    return jax.ops.segment_sum(src, seg, n)

class _Rng:

    def __init__(self, key):
        self._k = key

    def _next(self):
        self._k, sub = jax.random.split(self._k)
        return sub

    def normal(self, shape):
        return jax.random.normal(self._next(), shape, dtype=jnp.bfloat16)

    def randint(self, lo, hi, shape):
        return jax.random.randint(self._next(), shape, lo, hi, dtype=jnp.int32)

    def uniform(self, shape, lo=0.0, hi=1.0):
        return jax.random.uniform(self._next(), shape, jnp.bfloat16, lo, hi)

    def permutation(self, n):
        return jax.random.permutation(self._next(), n)
kernel_name = 'interleave_layers__sliding_local_dilated__mixer_gmlp__prompt'

def setup_inputs():
    _rng = _Rng(jax.random.key(int.from_bytes(__import__("os").urandom(4), "little")))
    _w = lambda a: (lambda t: t.astype(jnp.bfloat16) if jnp.issubdtype(t.dtype, jnp.floating) else t)(jnp.asarray(a))

    def _A_setup():
        B, S, D = (1, 2048, 576)
        return {'x': _w((lambda *s: _rng.normal(s) * 0.05)(B, S, D)), 'wqkv': _w((lambda *s: _rng.normal(s) * 0.05)(D, 3 * D)), 'wo': _w((lambda *s: _rng.normal(s) * 0.05)(D, D))}
    _A_in = _A_setup()

    def _B_setup():
        B, S, D, F = (1, 2048, 576, 4608)
        Fh = F // 2
        return {'x': _w((lambda *s: _rng.normal(s) * 0.05)(B, S, D)), 'w_in': _w((lambda *s: _rng.normal(s) * 0.05)(D, 2 * Fh)), 'w_sp': _w(0.01 * (lambda *s: _rng.normal(s) * 0.05)(S, S)), 'b_sp': _w(1.0 + 0.01 * (lambda *s: _rng.normal(s) * 0.05)(S)), 'w_out': _w((lambda *s: _rng.normal(s) * 0.05)(Fh, D))}
    _B_in = _B_setup()
    return {'A_x': _A_in['x'], 'A_wqkv': _A_in['wqkv'], 'A_wo': _A_in['wo'], 'B_x': _B_in['x'], 'B_w_in': _B_in['w_in'], 'B_w_sp': _B_in['w_sp'], 'B_b_sp': _B_in['b_sp'], 'B_w_out': _B_in['w_out']}

def reference(A_x, A_wqkv, A_wo, B_x, B_w_in, B_w_sp, B_b_sp, B_w_out):

    def _A_ref(x, wqkv, wo):
        B, S, D = x.shape
        H = 32
        Dh = D // H
        W, dil = (8, 2)
        qkv = (lambda x, *d: x.transpose(*d))((x @ wqkv).reshape(B, S, 3, H, Dh), 2, 0, 3, 1, 4)
        q, k, v = (qkv[0], qkv[1], qkv[2])
        scale = Dh ** (-0.5)
        pos = jnp.arange(S)
        off = jnp.arange(W) * dil
        idx = pos[:, None] - off[None, :]
        mask = idx >= 0
        idx_c = jnp.where(mask, idx, 0).reshape(-1)
        kg = k[:, :, idx_c, :].reshape(B, H, S, W, Dh)
        vg = v[:, :, idx_c, :].reshape(B, H, S, W, Dh)
        logits = jnp.einsum('bhsd,bhswd->bhsw', q, kg) * scale
        logits = jnp.where(mask[None, None, :, :], logits, -1000000000.0)
        attn = _softmax(logits, axis=-1)
        o = jnp.einsum('bhsw,bhswd->bhsd', attn, vg)
        return (lambda x, *d: x.transpose(*d))(o, 0, 2, 1, 3).reshape(B, S, D) @ wo

    def _B_ref(x, w_in, w_sp, b_sp, w_out):
        B, S, D = x.shape
        F = w_in.shape[-1]
        Fh = F // 2
        z = _gelu(jnp.einsum('bsd,df->bsf', x, w_in))
        z1 = z[..., :Fh].copy()
        z2 = _layernorm(z[..., Fh:], axis=-1)
        g = jnp.einsum('ts,bsf->btf', w_sp, z2) + b_sp[None, :, None]
        return jnp.einsum('bsf,fd->bsd', z1 * g, w_out)
    x = A_x
    x = x + _A_ref(_layernorm(x, axis=-1), A_wqkv, A_wo)
    x = x + _B_ref(_layernorm(x, axis=-1), B_w_in, B_w_sp, B_b_sp, B_w_out)
    x = x + _A_ref(_layernorm(x, axis=-1), A_wqkv, A_wo)
    x = x + _B_ref(_layernorm(x, axis=-1), B_w_in, B_w_sp, B_b_sp, B_w_out)
    return x
```

```python
import jax
import jax.numpy as jnp
from jax import lax
import jax.experimental.pallas as pl
import jax.experimental.pallas.tpu as pltpu

S, D, H, DH, W, DP, FH = 2048, 576, 32, 18, 8, 640, 2304
M1 = 512
M2 = 512
PAD = 16
F32, BF = jnp.float32, jnp.bfloat16


def _ln(x):
    m = jnp.mean(x, axis=-1, keepdims=True)
    c = x - m
    v = jnp.mean(c * c, axis=-1, keepdims=True)
    return c * lax.rsqrt(v + 1e-5)


def _gelu(x):
    t = jnp.tanh(x * (0.7978845608028654 + (0.7978845608028654 * 0.044715) * (x * x)))
    h = 0.5 * x
    return h + h * t


def _dot(a, b):
    return jnp.dot(a, b, preferred_element_type=F32)


def _kernel(x_ref, wq_in, wo_in, b_ref, win_h, wsp_h, wout_h, o_ref,
            xs, kb, vb, z1, z2, win, wsp, wout, sem, woutT, wqkv_ref, wo_ref, bt, xnb):
    c_in = pltpu.make_async_copy(win_h, win, sem.at[0])
    c_sp = pltpu.make_async_copy(wsp_h, wsp, sem.at[1])
    c_out = pltpu.make_async_copy(wout_h, woutT, sem.at[2])
    c_in.start()
    c_sp.start()
    c_out.start()
    xs[...] = x_ref[...].astype(F32).T
    bt[...] = jnp.broadcast_to(b_ref[...].astype(F32), (128, S)).T
    i = lax.broadcasted_iota(jnp.int32, (D, DP), 0)
    j = lax.broadcasted_iota(jnp.int32, (D, DP), 1)
    P = jnp.where((i == (j & 31) * DH + (j >> 5)) & (j < D), 1.0, 0.0).astype(BF)
    for t in range(3):
        wqkv_ref[t] = _dot(wq_in[:, t * D:(t + 1) * D], P).astype(BF)
    i = lax.broadcasted_iota(jnp.int32, (DP, D), 1)
    j = lax.broadcasted_iota(jnp.int32, (DP, D), 0)
    PT = jnp.where((i == (j & 31) * DH + (j >> 5)) & (j < D), 1.0, 0.0).astype(BF)
    wo_ref[...] = _dot(PT, wo_in[...]).astype(BF)
    c_in.wait()

    def layer(l, _):
        kb[0:PAD, :] = jnp.zeros((PAD, DP), F32)
        vb[0:PAD, :] = jnp.zeros((PAD, DP), F32)

        def pa(c):
            r0 = pl.multiple_of(c * M1, M1)
            rows = pl.ds(r0, M1)
            x = xs[rows, :]
            xn = _ln(x).astype(BF)
            kb[PAD:, :] = _dot(xn, wqkv_ref[1])
            vb[PAD:, :] = _dot(xn, wqkv_ref[2])
            q = _dot(xn, wqkv_ref[0]) * (DH ** -0.5)
            pos = r0 + lax.broadcasted_iota(jnp.int32, (M1, 128), 0)
            ls = []
            for w in range(W):
                st = PAD - 2 * w
                s = None
                for j in range(5):
                    sl = slice(j * 128, (j + 1) * 128)
                    p = q[:, sl] * kb[st:st + M1, sl]
                    s = p if s is None else s + p
                s = s + pltpu.roll(s, 64, 1)
                s = s + pltpu.roll(s, 32, 1)
                if w:
                    s = jnp.where(pos >= 2 * w, s, -1e9)
                ls.append(s)
            m = ls[0]
            for s in ls[1:]:
                m = jnp.maximum(m, s)
            es = [jnp.exp(s - m) for s in ls]
            t = es[0]
            for e in es[1:]:
                t = t + e
            r = 1.0 / t
            os_ = []
            for j in range(5):
                sl = slice(j * 128, (j + 1) * 128)
                a = None
                for w in range(W):
                    st = PAD - 2 * w
                    p = es[w] * vb[st:st + M1, sl]
                    a = p if a is None else a + p
                os_.append((a * r).astype(BF))
            o = jnp.concatenate(os_, axis=1)
            kb[0:PAD, :] = kb[M1:M1 + PAD, :]
            vb[0:PAD, :] = vb[M1:M1 + PAD, :]
            x = x + _dot(o, wo_ref[...])
            xs[rows, :] = x
            xnb[rows, :] = _ln(x).astype(BF)

        def pb(c):
            rows = pl.ds(pl.multiple_of(c * M1, M1), M1)
            xn = xnb[rows, :]
            zb = _gelu(_dot(xn, win[:, FH:]))
            z2[rows, :] = _ln(zb).astype(BF)
            z1[rows, :] = _gelu(_dot(xn, win[:, :FH])).astype(BF)

        def p1(c, _):
            pb(c - 1)
            pa(c)
            return 0

        pa(0)
        lax.fori_loop(1, S // M1, p1, 0)
        pb(S // M1 - 1)

        @pl.when(l == 0)
        def _():
            c_sp.wait()
            c_out.wait()
            wout[...] = woutT[...].T

        def p2(c, _):
            rows = pl.ds(pl.multiple_of(c * M2, M2), M2)
            g = _dot(wsp[rows, :], z2[...]) + jnp.tile(bt[rows, :], (1, FH // 128))
            u = (z1[rows, :].astype(F32) * g).astype(BF)
            xs[rows, :] = xs[rows, :] + _dot(u, wout[...])
            return 0

        lax.fori_loop(0, S // M2, p2, 0)
        return 0

    lax.fori_loop(0, 2, layer, 0)
    o_ref[...] = xs[...].T.astype(BF)


@jax.jit
def pallas_interleave_layers__sliding_local_dilated__mixer_gmlp__prompt_kernel(
    A_x, A_wqkv, A_wo, B_x, B_w_in, B_w_sp, B_b_sp, B_w_out,
):
    vm = pl.BlockSpec(memory_space=pltpu.VMEM)
    hb = pl.BlockSpec(memory_space=pl.ANY)
    out = pl.pallas_call(
        _kernel,
        in_specs=[vm, vm, vm, vm, hb, hb, hb],
        out_specs=vm,
        out_shape=jax.ShapeDtypeStruct((D, S), BF),
        scratch_shapes=[
            pltpu.VMEM((S, D), F32),
            pltpu.VMEM((M1 + PAD, DP), F32),
            pltpu.VMEM((M1 + PAD, DP), F32),
            pltpu.VMEM((S, FH), BF),
            pltpu.VMEM((S, FH), BF),
            pltpu.VMEM((D, 2 * FH), BF),
            pltpu.VMEM((S, S), BF),
            pltpu.VMEM((FH, D), BF),
            pltpu.SemaphoreType.DMA((3,)),
            pltpu.VMEM((D, FH), BF),
            pltpu.VMEM((3, D, DP), BF),
            pltpu.VMEM((DP, D), BF),
            pltpu.VMEM((S, 128), F32),
            pltpu.VMEM((S, D), BF),
        ],
        compiler_params=pltpu.CompilerParams(vmem_limit_bytes=120 * 1024 * 1024),
    )(A_x.reshape(S, D).T, A_wqkv, A_wo, B_b_sp.reshape(1, S), B_w_in, B_w_sp, B_w_out.T)
    return out.T.reshape(1, S, D)
```

```python
import jax
import jax.numpy as jnp
from jax import lax
import jax.experimental.pallas as pl
import jax.experimental.pallas.tpu as pltpu

S, D, H, DH, W, FH = 2048, 576, 32, 18, 8, 2304
T = 512
NC = S // T
NP = 4
FP = FH // NP
F32, BF = jnp.float32, jnp.bfloat16


def _ln0(x):
    m = jnp.mean(x, axis=0, keepdims=True)
    c = x - m
    v = jnp.mean(c * c, axis=0, keepdims=True)
    return c * lax.rsqrt(v + 1e-5)


def _gelu2(x):
    t = jnp.tanh(x * (0.7978845608028654 + (0.7978845608028654 * 0.044715) * (x * x)))
    return x + x * t


def _dot(a, b):
    return jnp.dot(a, b, preferred_element_type=F32)


def _dot_nt(a, b):
    return lax.dot_general(a, b, (((1,), (1,)), ((), ())), preferred_element_type=F32)


def _kernel(b_ref, x_h, wq_h, wo_h, win_h, wsp_h, wout_h, o_h,
            xs, xio, wq_in, wo_in, win_in, wq, wo, win, wsp, wout,
            qb, kb, vb, ob, xnb, zf, z1, z2, ub, tmp, sem, xsem):
    xin = [pltpu.make_async_copy(x_h.at[:, c * T:(c + 1) * T], xio.at[c], xsem.at[c])
           for c in range(NC)]
    c_q = pltpu.make_async_copy(wq_h, wq_in, sem.at[0])
    c_o = pltpu.make_async_copy(wo_h, wo_in, sem.at[1])
    c_in = pltpu.make_async_copy(win_h, win_in, sem.at[2])
    c_sp = pltpu.make_async_copy(wsp_h, wsp, sem.at[3])
    c_out = pltpu.make_async_copy(wout_h, wout, sem.at[4])
    c_o.start()
    c_q.start()
    xin[0].start()

    def put(v):
        for k in range(5):
            wd = min(128, D - k * 128)
            tmp[k, 0:v.shape[0], 0:wd] = v[:, k * 128:k * 128 + wd]

    def heads(r):
        return jnp.concatenate(
            [tmp[k, pl.ds(r, H, stride=DH), :][:, 0:min(128, D - k * 128)]
             for k in range(5)], axis=1)

    c_o.wait()
    put(wo_in[...].astype(F32))
    wo[...] = jnp.concatenate(
        [heads(d) for d in range(DH)], axis=0).T.astype(BF)
    c_q.wait()
    c_in.start()
    for c in range(1, NC):
        xin[c].start()
    put(wq_in[...].astype(F32).T)
    for t in range(3):
        for d in range(DH):
            r = t * D + d * H
            wq[r:r + H, :] = heads(t * D + d).astype(BF)
    xin[0].wait()
    xs[0] = xio[0].astype(F32)

    lane = lax.broadcasted_iota(jnp.int32, (8, 128), 1)

    def shifted(ref, r, tl, w):
        cur = ref[r:r + 8, (tl + 1) * 128:(tl + 2) * 128]
        if w == 0:
            return cur
        prev = ref[r:r + 8, tl * 128:(tl + 1) * 128]
        return pltpu.roll(jnp.where(lane >= 128 - 2 * w, prev, cur), 2 * w, 1)

    def a_qkv(c):
        xn = _ln0(xs[c]).astype(BF)
        kb[:, 128:] = _dot(wq[D:2 * D, :], xn)
        qb[...] = _dot(wq[0:D, :], xn) * (DH ** -0.5)
        vb[:, 128:] = _dot(wq[2 * D:, :], xn)

    def a_att(c, tl, hp):
        outs = []
        for hg in (2 * hp, 2 * hp + 1):
            ls = [None] * W
            for d in range(DH):
                r = d * H + hg * 8
                q = qb[r:r + 8, tl * 128:(tl + 1) * 128]
                for w in range(W):
                    p = q * shifted(kb, r, tl, w)
                    ls[w] = p if d == 0 else ls[w] + p
            if tl == 0:
                pos = c * T + lane
                ls = [s if w == 0 else jnp.where(pos >= 2 * w, s, -1e9)
                      for w, s in enumerate(ls)]
            m = ls[0]
            for s in ls[1:]:
                m = jnp.maximum(m, s)
            es = [jnp.exp(s - m) for s in ls]
            t = es[0]
            for e in es[1:]:
                t = t + e
            rc = 1.0 / t
            o = []
            for d in range(DH):
                r = d * H + hg * 8
                a = es[0] * shifted(vb, r, tl, 0)
                for w in range(1, W):
                    a = a + es[w] * shifted(vb, r, tl, w)
                o.append(a * rc)
            outs.append(o)
        for d in range(DH):
            r = d * H + hp * 16
            ob[r:r + 16, tl * 128:(tl + 1) * 128] = jnp.concatenate(
                [outs[0][d], outs[1][d]], axis=0).astype(BF)

    def a_out(c):
        kb[:, 0:128] = kb[:, T:]
        vb[:, 0:128] = vb[:, T:]
        x = xs[c] + _dot(wo[...], ob[...])
        xs[c] = x
        xnb[c] = _ln0(x).astype(BF)

    units = [(tl, hp) for tl in range(T // 128) for hp in range(2)]

    def b_steps(c):
        st = {}

        def z2p(p):
            z = _gelu2(_dot(win[FH + p * FP:FH + (p + 1) * FP, :], xnb[c]))
            if p == 0:
                st['m0'] = jnp.mean(z, axis=0, keepdims=True)
            z = z - st['m0']
            zf[p * FP:(p + 1) * FP, :] = z
            s = jnp.sum(z, axis=0, keepdims=True)
            v = jnp.sum(z * z, axis=0, keepdims=True)
            st['s'] = s if p == 0 else st['s'] + s
            st['v'] = v if p == 0 else st['v'] + v

        def z1p(p):
            z = _gelu2(_dot(win[p * FP:(p + 1) * FP, :], xnb[c]))
            z1[c, p * FP:(p + 1) * FP, :] = z.astype(BF)
            if p == 0:
                st['m'] = st['s'] * (1.0 / FH)
                var = jnp.maximum(st['v'] * (1.0 / FH) - st['m'] * st['m'], 0.0)
                st['r'] = 0.5 * lax.rsqrt(var + 4e-5)
            a = p * FP
            z2[a:a + FP, pl.ds(pl.multiple_of(c * T, T), T)] = (
                (zf[a:a + FP, :] - st['m']) * st['r']).astype(BF)

        return ([lambda p=p: z2p(p) for p in range(NP)]
                + [lambda p=p: z1p(p) for p in range(NP)])

    def layer(l, _):
        kb[:, 0:128] = jnp.zeros((D, 128), F32)
        vb[:, 0:128] = jnp.zeros((D, 128), F32)
        with jax.named_scope('pa0'):
            a_qkv(0)
            for u in units:
                a_att(0, *u)
            a_out(0)

        @pl.when(l == 0)
        def _():
            c_in.wait()
            c_sp.start()
            c_out.start()
            for c in range(1, NC):
                xin[c].wait()
                xs[c] = xio[c].astype(F32)
            win[...] = win_in[...].T

        def p1(c, _):
            bs = b_steps(c - 1)
            bs[0]()
            a_qkv(c)
            mid = bs[1:-1]
            for k, u in enumerate(units):
                a_att(c, *u)
                for q in mid[k * len(mid) // len(units):(k + 1) * len(mid) // len(units)]:
                    q()
            a_out(c)
            bs[-1]()
            return 0

        with jax.named_scope('p1'):
            lax.fori_loop(1, NC, p1, 0)
        with jax.named_scope('pbl'):
            for q in b_steps(NC - 1):
                q()

        @pl.when(l == 0)
        def _():
            c_sp.wait()
            c_out.wait()

        def p2(c, _):
            col = pl.ds(pl.multiple_of(c * T, T), T)
            bias = 0.5 * b_ref[:, col].astype(F32)
            for a in range(0, FH, 768):
                g = _dot_nt(z2[a:a + 768, :], wsp[col, :]) + bias
                ub[a:a + 768, :] = (z1[c, a:a + 768, :].astype(F32) * g).astype(BF)
            x = xs[c] + _dot(wout[...], ub[...])
            xs[c] = x
            xio[c] = x.astype(BF)

            @pl.when(l == 1)
            def _():
                pltpu.make_async_copy(xio.at[c], o_h.at[:, col], xsem.at[c]).start()
            return 0

        with jax.named_scope('p2'):
            lax.fori_loop(0, NC, p2, 0)
        return 0

    with jax.named_scope('layers'):
        lax.fori_loop(0, 2, layer, 0)
    for c in range(NC):
        pltpu.make_async_copy(xio.at[c], o_h.at[:, c * T:(c + 1) * T], xsem.at[c]).wait()


@jax.jit
def pallas_interleave_layers__sliding_local_dilated__mixer_gmlp__prompt_kernel(
    A_x, A_wqkv, A_wo, B_x, B_w_in, B_w_sp, B_b_sp, B_w_out,
):
    vm = pl.BlockSpec(memory_space=pltpu.VMEM)
    hb = pl.BlockSpec(memory_space=pl.ANY)
    V = pltpu.VMEM
    out = pl.pallas_call(
        _kernel,
        in_specs=[vm, hb, hb, hb, hb, hb, hb],
        out_specs=hb,
        out_shape=jax.ShapeDtypeStruct((D, S), BF),
        scratch_shapes=[
            V((NC, D, T), F32), V((NC, D, T), BF),
            V((D, 3 * D), BF), V((D, D), BF), V((D, 2 * FH), BF),
            V((3 * D, D), BF), V((D, D), BF), V((2 * FH, D), BF),
            V((S, S), BF), V((D, FH), BF),
            V((D, T), F32), V((D, T + 128), F32), V((D, T + 128), F32),
            V((D, T), BF), V((NC, D, T), BF),
            V((FH, T), F32), V((NC, FH, T), BF), V((FH, S), BF), V((FH, T), BF),
            V((5, 3 * D, 128), F32),
            pltpu.SemaphoreType.DMA((5,)), pltpu.SemaphoreType.DMA((NC,)),
        ],
        compiler_params=pltpu.CompilerParams(vmem_limit_bytes=120 * 1024 * 1024),
    )(B_b_sp.reshape(1, S), A_x.reshape(S, D).T, A_wqkv, A_wo, B_w_in, B_w_sp, B_w_out.T)
    return out.T.reshape(1, S, D)
```
